```python
import jax
import jax.numpy as jnp

def _softmax(x, axis=-1):
    return jax.nn.softmax(x, axis=axis)
def _gelu(x):
    return jax.nn.gelu(x, approximate=True)
def _silu(x):
    return jax.nn.silu(x)
def _sigmoid(x):
    return jax.nn.sigmoid(x)
def _layernorm(x, axis=-1, eps=1e-5):
    m = jnp.mean(x, axis=axis, keepdims=True)
    v = jnp.var(x, axis=axis, keepdims=True)
    return (x - m) / jnp.sqrt(v + eps)
def _scatter_add(tgt, idx, src, axis=0):
    return tgt.at[idx].add(src)
def _segment_sum(src, seg, n):
    return jax.ops.segment_sum(src, seg, n)
class _Rng:
    def __init__(self, key):
        self._k = key
    def _next(self):
        self._k, sub = jax.random.split(self._k)
        return sub
    def normal(self, shape):
        return jax.random.normal(self._next(), shape, dtype=jnp.bfloat16)
    def randint(self, lo, hi, shape):
        return jax.random.randint(self._next(), shape, lo, hi, dtype=jnp.int32)
    def uniform(self, shape, lo=0.0, hi=1.0):
        return jax.random.uniform(self._next(), shape, jnp.bfloat16, lo, hi)
    def permutation(self, n):
        return jax.random.permutation(self._next(), n)


kernel_name = 'recurrent_scan__sliding_block_cached__glu_gated_glu__decode'

def setup_inputs():
    _rng = _Rng(jax.random.key(int.from_bytes(__import__("os").urandom(4), "little")))
    _w = (lambda a: (lambda t: t.astype(jnp.bfloat16) if jnp.issubdtype(t.dtype, jnp.floating) else t)(jnp.asarray(a)))
    def _A_setup():
        B, Sq, D = 1, 1, 576
        Hq, Hkv, Sk, Dh = 32, 16, 65536, 128
        assert Hq % Hkv == 0, (Hq, Hkv)
        return {
            "x": _w((lambda *s: _rng.normal(s) * 0.05)(B, Sq, D)),
            "k_cache": _w((lambda *s: _rng.normal(s) * 0.05)(B, Hkv, Sk, Dh)),
            "v_cache": _w((lambda *s: _rng.normal(s) * 0.05)(B, Hkv, Sk, Dh)),
            "wq": _w((lambda *s: _rng.normal(s) * 0.05)(D, Hq * Dh) * (D ** -0.5)),
            "wo": _w((lambda *s: _rng.normal(s) * 0.05)(Hq * Dh, D) * ((Hq * Dh) ** -0.5)),
        }
    _A_in = _A_setup()

    def _B_setup():
        B, S, D, F = 1, 1, 576, 4608
        return {
            "x": _w((lambda *s: _rng.normal(s) * 0.05)(B, S, D)),
            "w_gate": _w((lambda *s: _rng.normal(s) * 0.05)(D, F)),
            "w_up": _w((lambda *s: _rng.normal(s) * 0.05)(D, F)),
            "w_down": _w((lambda *s: _rng.normal(s) * 0.05)(F, D)),
        }
    _B_in = _B_setup()

    return {
        "A_x": _A_in["x"],
        "A_k_cache": _A_in["k_cache"],
        "A_v_cache": _A_in["v_cache"],
        "A_wq": _A_in["wq"],
        "A_wo": _A_in["wo"],
        "B_x": _B_in["x"],
        "B_w_gate": _B_in["w_gate"],
        "B_w_up": _B_in["w_up"],
        "B_w_down": _B_in["w_down"],
    }

def reference(A_x, A_k_cache, A_v_cache, A_wq, A_wo, B_x, B_w_gate, B_w_up, B_w_down):
    def _A_ref(x, k_cache, v_cache, wq, wo):
        B, Sq, D = x.shape
        Hq, Dh = 32, 128
        Hkv, Sk = k_cache.shape[1], k_cache.shape[2]
        W = min(4096, max(256, Sk // 4))
        rep = Hq // Hkv
        q = (lambda x, *d: x.transpose(*d))((x @ wq).reshape(B, Sq, Hq, Dh), 0, 2, 1, 3)
        k = jnp.repeat(k_cache[:, :, Sk - W:, :], rep, axis=1)
        v = jnp.repeat(v_cache[:, :, Sk - W:, :], rep, axis=1)
        scores = jnp.einsum("bhqd,bhkd->bhqk", q, k) * (Dh ** -0.5)
        p = _softmax(scores, axis=-1)
        o = jnp.einsum("bhqk,bhkd->bhqd", p, v)
        return (lambda x, *d: x.transpose(*d))(o, 0, 2, 1, 3).reshape(B, Sq, Hq * Dh) @ wo

    def _B_ref(x, w_gate, w_up, w_down):
        g = jnp.einsum("bsd,df->bsf", x, w_gate)
        u = jnp.einsum("bsd,df->bsf", x, w_up)
        h = _sigmoid(g) * u
        return jnp.einsum("bsf,fd->bsd", h, w_down)

    x = A_x
    xn = _layernorm(x, axis=-1)
    s = _A_ref(xn, A_k_cache, A_v_cache, A_wq, A_wo)
    g = _silu(_B_ref(xn, B_w_gate, B_w_up, B_w_down))
    return x + s * g
```

```python
import jax
import jax.numpy as jnp
import jax.experimental.pallas as pl
import jax.experimental.pallas.tpu as pltpu

_NT = (((1,), (1,)), ((), ()))
_NN = (((1,), (0,)), ((), ()))


def _build(D, HQ, HKV, SK, DH, F):
    W = min(4096, max(256, SK // 4))
    REP = HQ // HKV
    HD = HQ * DH
    f32, bf16 = jnp.float32, jnp.bfloat16
    WD_ROWS = 64
    n_wd = D // WD_ROWS
    S_X, S_WQ, S_WO, S_WG, S_WU = 0, 1, 2, 3, 4
    S_K = 5
    S_V = S_K + HKV
    S_WD = S_V + HKV
    NSEM = S_WD + n_wd

    def kernel(x_hbm, wq_hbm, k_hbm, v_hbm, wo_hbm, wg_hbm, wu_hbm, wd_hbm, out_ref,
               x_v, wq_v, k_v, v_v, wo_v, wg_v, wu_v, wd_v, q_s, o_s, sems):
        def cp(src, dst, s):
            return pltpu.make_async_copy(src, dst, sems.at[s])

        def k_copy(h):
            return cp(k_hbm.at[0, h, pl.ds(SK - W, W)], k_v.at[h], S_K + h)

        def v_copy(h):
            return cp(v_hbm.at[0, h, pl.ds(SK - W, W)], v_v.at[h], S_V + h)

        def wd_copy(i):
            return cp(wd_hbm.at[pl.ds(i * WD_ROWS, WD_ROWS)],
                      wd_v.at[pl.ds(i * WD_ROWS, WD_ROWS)], S_WD + i)

        x_cp = cp(x_hbm, x_v, S_X)
        wq_cp = cp(wq_hbm, wq_v, S_WQ)
        wo_cp = cp(wo_hbm, wo_v, S_WO)
        wg_cp = cp(wg_hbm, wg_v, S_WG)
        wu_cp = cp(wu_hbm, wu_v, S_WU)

        x_cp.start()
        wq_cp.start()
        for h in range(HKV):
            k_copy(h).start()
            v_copy(h).start()
        wo_cp.start()
        wg_cp.start()
        wu_cp.start()
        for i in range(n_wd):
            wd_copy(i).start()

        x_cp.wait()
        x = x_v[0].astype(f32)
        mu = jnp.mean(x, axis=-1, keepdims=True)
        xc = x - mu
        var = jnp.mean(xc * xc, axis=-1, keepdims=True)
        xn = xc * jax.lax.rsqrt(var + 1e-5)
        xn8 = jnp.broadcast_to(xn, (8, D)).astype(bf16)

        wq_cp.wait()
        q = jax.lax.dot_general(xn8, wq_v[...], _NN, preferred_element_type=f32)
        q = q * (DH ** -0.5)
        row = jax.lax.broadcasted_iota(jnp.int32, (8, DH), 0)
        for h in range(HKV):
            qh = q[:, (REP * h) * DH:(REP * h + 1) * DH]
            for r in range(1, REP):
                qh = jnp.where(row == r, q[:, (REP * h + r) * DH:(REP * h + r + 1) * DH], qh)
            q_s[h] = qh

        def head(h, carry):
            k_copy(h).wait()
            qh = q_s[h].astype(bf16)
            s = jax.lax.dot_general(qh, k_v[h], _NT, preferred_element_type=f32)
            m = jnp.max(s, axis=-1, keepdims=True)
            p = jnp.exp(s - m)
            l = jnp.sum(p, axis=-1, keepdims=True)
            v_copy(h).wait()
            o = jax.lax.dot_general(p.astype(bf16), v_v[h], _NN, preferred_element_type=f32)
            o_s[h] = o / l
            return carry

        jax.lax.fori_loop(0, HKV, head, 0)

        o_flat = jnp.concatenate(
            [o_s[h][r:r + 1, :] for h in range(HKV) for r in range(REP)], axis=1)
        o8 = jnp.broadcast_to(o_flat, (8, HD)).astype(bf16)
        wo_cp.wait()
        s_att = jax.lax.dot_general(o8, wo_v[...], _NT, preferred_element_type=f32)

        wg_cp.wait()
        g = jax.lax.dot_general(xn8, wg_v[...], _NN, preferred_element_type=f32)
        wu_cp.wait()
        u = jax.lax.dot_general(xn8, wu_v[...], _NN, preferred_element_type=f32)
        hh = (jax.nn.sigmoid(g) * u).astype(bf16)
        ys = []
        for i in range(n_wd):
            wd_copy(i).wait()
            ys.append(jax.lax.dot_general(hh, wd_v[pl.ds(i * WD_ROWS, WD_ROWS), :], _NT,
                                          preferred_element_type=f32))
        y = jnp.concatenate(ys, axis=1)
        res = x + s_att[0:1, :] * (y[0:1, :] * jax.nn.sigmoid(y[0:1, :]))
        out_ref[0] = res.astype(out_ref.dtype)

    scratch = [
        pltpu.VMEM((1, 1, D), bf16),
        pltpu.VMEM((D, HD), bf16),
        pltpu.VMEM((HKV, W, DH), bf16),
        pltpu.VMEM((HKV, W, DH), bf16),
        pltpu.VMEM((D, HD), bf16),
        pltpu.VMEM((D, F), bf16),
        pltpu.VMEM((D, F), bf16),
        pltpu.VMEM((D, F), bf16),
        pltpu.VMEM((HKV, 8, DH), f32),
        pltpu.VMEM((HKV, 8, DH), f32),
        pltpu.SemaphoreType.DMA((NSEM,)),
    ]
    return kernel, scratch


@jax.jit
def pallas_recurrent_scan__sliding_block_cached__glu_gated_glu__decode_kernel(
    A_x: jax.Array,
    A_k_cache: jax.Array,
    A_v_cache: jax.Array,
    A_wq: jax.Array,
    A_wo: jax.Array,
    B_x: jax.Array,
    B_w_gate: jax.Array,
    B_w_up: jax.Array,
    B_w_down: jax.Array,
):
    _, _, D = A_x.shape
    _, HKV, SK, DH = A_k_cache.shape
    HQ = A_wq.shape[1] // DH
    F = B_w_gate.shape[1]
    kernel, scratch = _build(D, HQ, HKV, SK, DH, F)
    return pl.pallas_call(
        kernel,
        out_shape=jax.ShapeDtypeStruct(A_x.shape, A_x.dtype),
        in_specs=[pl.BlockSpec(memory_space=pl.ANY)] * 8,
        out_specs=pl.BlockSpec(memory_space=pltpu.VMEM),
        scratch_shapes=scratch,
        compiler_params=pltpu.CompilerParams(vmem_limit_bytes=100 * 1024 * 1024, disable_semaphore_checks=True),
    )(A_x, A_wq, A_k_cache, A_v_cache, A_wo.T, B_w_gate, B_w_up, B_w_down.T)
```

```python
import jax
import jax.numpy as jnp
import jax.experimental.pallas as pl
import jax.experimental.pallas.tpu as pltpu

_NT = (((1,), (1,)), ((), ()))
_NN = (((1,), (0,)), ((), ()))
_LANES = 128
_SUB = 8


def _tree_sum(xs):
    xs = list(xs)
    while len(xs) > 1:
        nxt = [xs[i] + xs[i + 1] for i in range(0, len(xs) - 1, 2)]
        if len(xs) % 2:
            nxt.append(xs[-1])
        xs = nxt
    return xs[0]


def _build(D, HQ, HKV, SK, DH, F):
    W = min(4096, max(256, SK // 4))
    REP = HQ // HKV
    HD = HQ * DH
    f32, bf16 = jnp.float32, jnp.bfloat16
    assert REP <= _SUB and D == 576 and HD % _LANES == 0

    R_TAIL = 512
    N_TAIL = D - R_TAIL
    mxu_rows = ((0, 256), (256, 384), (384, 448), (448, 512))
    vpu_rows = ((512, 552), (552, 568), (568, 576))
    wo_rows = mxu_rows + vpu_rows

    S_X, S_WQ, S_WG, S_WU, S_WD = 0, 1, 2, 3, 4
    S_K = 5
    S_V = S_K + HKV
    S_WO = S_V + HKV
    NSEM = S_WO + len(wo_rows)

    def kernel(x_hbm, wq_hbm, k_hbm, v_hbm, wo_hbm, wg_hbm, wu_hbm, wd_hbm, out_ref,
               x_v, wq_v, k_v, v_v, wo_v, wg_v, wu_v, wd_v, q_s, o_s, of_s):

        def main(sems):
            def cp(src, dst, s):
                return pltpu.make_async_copy(src, dst, sems.at[s])

            def k_copy(h):
                return cp(k_hbm.at[0, h, pl.ds(SK - W, W)], k_v.at[h], S_K + h)

            def v_copy(h):
                return cp(v_hbm.at[0, h, pl.ds(SK - W, W)], v_v.at[h], S_V + h)

            def wo_copy(i):
                r0, r1 = wo_rows[i]
                return cp(wo_hbm.at[pl.ds(r0, r1 - r0)], wo_v.at[pl.ds(r0, r1 - r0)], S_WO + i)

            x_cp = cp(x_hbm, x_v, S_X)
            wq_cp = cp(wq_hbm, wq_v, S_WQ)
            wg_cp = cp(wg_hbm, wg_v, S_WG)
            wu_cp = cp(wu_hbm, wu_v, S_WU)
            wd_cp = cp(wd_hbm, wd_v, S_WD)

            x_cp.start()
            wq_cp.start()
            for h in range(HKV):
                k_copy(h).start()
                v_copy(h).start()
            wg_cp.start()
            wu_cp.start()
            wd_cp.start()
            for i in range(len(wo_rows)):
                wo_copy(i).start()

            x_cp.wait()
            x = x_v[0].astype(f32)
            mu = jnp.mean(x, axis=-1, keepdims=True)
            xc = x - mu
            var = jnp.mean(xc * xc, axis=-1, keepdims=True)
            xn = xc * jax.lax.rsqrt(var + 1e-5)
            xn8 = jnp.broadcast_to(xn, (_SUB, D)).astype(bf16)
            x8 = jnp.broadcast_to(x, (_SUB, D))

            wq_cp.wait()
            q = jax.lax.dot_general(xn8, wq_v[...], _NN, preferred_element_type=f32)
            q = q * (DH ** -0.5)
            row = jax.lax.broadcasted_iota(jnp.int32, (_SUB, DH), 0)
            for h in range(HKV):
                qh = q[:, (REP * h) * DH:(REP * h + 1) * DH]
                for r in range(1, REP):
                    qh = jnp.where(row == r, q[:, (REP * h + r) * DH:(REP * h + r + 1) * DH], qh)
                q_s[h] = qh

            def head(h, carry):
                k_copy(h).wait()
                s = jax.lax.dot_general(q_s[h].astype(bf16), k_v[h], _NT,
                                        preferred_element_type=f32)
                m = jnp.max(s, axis=-1, keepdims=True)
                p = jnp.exp(s - m)
                l = jnp.sum(p, axis=-1, keepdims=True)
                v_copy(h).wait()
                o = jax.lax.dot_general(p.astype(bf16), v_v[h], _NN,
                                        preferred_element_type=f32)
                o_s[h] = o / l
                return carry

            jax.lax.fori_loop(0, HKV, head, 0)

            o_flat = jnp.concatenate(
                [o_s[h][r:r + 1, :] for h in range(HKV) for r in range(REP)], axis=1)
            o8 = jnp.broadcast_to(o_flat, (_SUB, HD)).astype(bf16)
            of_s[...] = o8.astype(f32)

            wg_cp.wait()
            g = jax.lax.dot_general(xn8, wg_v[...], _NN, preferred_element_type=f32)
            wu_cp.wait()
            u = jax.lax.dot_general(xn8, wu_v[...], _NN, preferred_element_type=f32)
            hh = (jax.nn.sigmoid(g) * u).astype(bf16)
            wd_cp.wait()
            y = jax.lax.dot_general(hh, wd_v[...], _NT, preferred_element_type=f32)
            gate = y * jax.nn.sigmoid(y)

            parts = []
            for i, (r0, r1) in enumerate(mxu_rows):
                wo_copy(i).wait()
                parts.append(jax.lax.dot_general(o8, wo_v[pl.ds(r0, r1 - r0), :], _NT,
                                                 preferred_element_type=f32))
            s_head = jnp.concatenate(parts, axis=1)
            res = x8[:, 0:R_TAIL] + s_head * gate[:, 0:R_TAIL]
            out_ref[0, :, 0:R_TAIL] = res[0:1].astype(out_ref.dtype)

            lane = jax.lax.broadcasted_iota(jnp.int32, (_SUB, N_TAIL), 1)
            sub = jax.lax.broadcasted_iota(jnp.int32, (_SUB, N_TAIL), 0)

            def place(acc, r, part):
                tot = jnp.sum(part, axis=-1, keepdims=True)
                return jnp.where(lane == sub + (r - R_TAIL), tot, acc)

            acc = jnp.zeros((_SUB, N_TAIL), f32)
            pending = []
            for i, (r0, r1) in enumerate(vpu_rows):
                wo_copy(len(mxu_rows) + i).wait()
                for r, part in pending:
                    acc = place(acc, r, part)
                pending = []
                for r in range(r0, r1, _SUB):
                    w = wo_v[pl.ds(r, _SUB), :].astype(f32)
                    pending.append((r, _tree_sum(
                        [w[:, c:c + _LANES] * of_s[:, c:c + _LANES] for c in range(0, HD, _LANES)])))
            for r, part in pending:
                acc = place(acc, r, part)
            s_tail = jnp.sum(acc, axis=0, keepdims=True)
            res_t = x[:, R_TAIL:] + s_tail * gate[0:1, R_TAIL:]
            out_ref[0, :, R_TAIL:D] = res_t.astype(out_ref.dtype)

        pl.run_scoped(main, pltpu.SemaphoreType.DMA((NSEM,)))

    scratch = [
        pltpu.VMEM((1, 1, D), bf16),
        pltpu.VMEM((D, HD), bf16),
        pltpu.VMEM((HKV, W, DH), bf16),
        pltpu.VMEM((HKV, W, DH), bf16),
        pltpu.VMEM((D, HD), bf16),
        pltpu.VMEM((D, F), bf16),
        pltpu.VMEM((D, F), bf16),
        pltpu.VMEM((D, F), bf16),
        pltpu.VMEM((HKV, _SUB, DH), f32),
        pltpu.VMEM((HKV, _SUB, DH), f32),
        pltpu.VMEM((_SUB, HD), f32),
    ]
    return kernel, scratch


@jax.jit
def pallas_recurrent_scan__sliding_block_cached__glu_gated_glu__decode_kernel(
    A_x: jax.Array,
    A_k_cache: jax.Array,
    A_v_cache: jax.Array,
    A_wq: jax.Array,
    A_wo: jax.Array,
    B_x: jax.Array,
    B_w_gate: jax.Array,
    B_w_up: jax.Array,
    B_w_down: jax.Array,
):
    _, _, D = A_x.shape
    _, HKV, SK, DH = A_k_cache.shape
    HQ = A_wq.shape[1] // DH
    F = B_w_gate.shape[1]
    kernel, scratch = _build(D, HQ, HKV, SK, DH, F)
    return pl.pallas_call(
        kernel,
        out_shape=jax.ShapeDtypeStruct(A_x.shape, A_x.dtype),
        in_specs=[pl.BlockSpec(memory_space=pl.ANY)] * 8,
        out_specs=pl.BlockSpec(memory_space=pltpu.VMEM),
        scratch_shapes=scratch,
        compiler_params=pltpu.CompilerParams(vmem_limit_bytes=100 * 1024 * 1024),
    )(A_x, A_wq, A_k_cache, A_v_cache, A_wo.T, B_w_gate, B_w_up, B_w_down.T)
```

```python
import jax
import jax.numpy as jnp
import jax.experimental.pallas as pl
import jax.experimental.pallas.tpu as pltpu

_NT = (((1,), (1,)), ((), ()))
_NN = (((1,), (0,)), ((), ()))
_LANES = 128
_SUB = 8
_EPS_BF16 = 1.0013580322265625e-05


def _tree_sum(xs):
    xs = list(xs)
    while len(xs) > 1:
        nxt = [xs[i] + xs[i + 1] for i in range(0, len(xs) - 1, 2)]
        if len(xs) % 2:
            nxt.append(xs[-1])
        xs = nxt
    return xs[0]


def _build(D, HQ, HKV, SK, DH, F):
    W = min(4096, max(256, SK // 4))
    REP = HQ // HKV
    HD = HQ * DH
    f32, bf16 = jnp.float32, jnp.bfloat16
    assert REP <= _SUB and D == 576 and HD % _LANES == 0 and DH == 128
    sm_scale = 0.08837890625

    R_TAIL = 512
    N_TAIL = D - R_TAIL
    mxu_rows = ((0, 256), (256, 384), (384, 448), (448, 512))
    vpu_rows = ((512, 544), (544, 560), (560, 576))
    wo_rows = mxu_rows + vpu_rows

    S_X, S_WQ, S_WG, S_WU, S_WD = 0, 1, 2, 3, 4
    S_K = 5
    S_V = S_K + HKV
    S_WO = S_V + HKV
    NSEM = S_WO + len(wo_rows)

    def kernel(x_hbm, wq_hbm, k_hbm, v_hbm, wo_hbm, wg_hbm, wu_hbm, wd_hbm, out_ref,
               x_v, wq_v, k_v, v_v, wo_v, wg_v, wu_v, wd_v, q_s, o_s, of_s):

        def main(sems):
            def cp(src, dst, s):
                return pltpu.make_async_copy(src, dst, sems.at[s])

            def k_copy(h):
                return cp(k_hbm.at[0, h, pl.ds(SK - W, W)], k_v.at[h], S_K + h)

            def v_copy(h):
                return cp(v_hbm.at[0, h, pl.ds(SK - W, W)], v_v.at[h], S_V + h)

            def wo_copy(i):
                r0, r1 = wo_rows[i]
                return cp(wo_hbm.at[pl.ds(r0, r1 - r0)], wo_v.at[pl.ds(r0, r1 - r0)], S_WO + i)

            x_cp = cp(x_hbm, x_v, S_X)
            wq_cp = cp(wq_hbm, wq_v, S_WQ)
            wg_cp = cp(wg_hbm, wg_v, S_WG)
            wu_cp = cp(wu_hbm, wu_v, S_WU)
            wd_cp = cp(wd_hbm, wd_v, S_WD)

            x_cp.start()
            wq_cp.start()
            for h in range(HKV):
                k_copy(h).start()
                v_copy(h).start()
            wg_cp.start()
            wu_cp.start()
            wd_cp.start()
            for i in range(len(wo_rows)):
                wo_copy(i).start()

            def rnd(a):
                return a.astype(bf16).astype(f32)

            x_cp.wait()
            x = x_v[0].astype(f32)
            mu = jnp.mean(x, axis=-1, keepdims=True)
            xc = x - mu
            var = rnd(jnp.mean(xc * xc, axis=-1, keepdims=True))
            std = rnd(jnp.sqrt(rnd(var + _EPS_BF16)))
            xn = rnd(x - rnd(mu)) / std
            xn8 = jnp.broadcast_to(xn, (_SUB, D)).astype(bf16)
            x8 = jnp.broadcast_to(x, (_SUB, D))

            wq_cp.wait()
            q = jax.lax.dot_general(xn8, wq_v[...], _NN, preferred_element_type=f32)
            row = jax.lax.broadcasted_iota(jnp.int32, (_SUB, DH), 0)
            for h in range(HKV):
                qh = q[:, (REP * h) * DH:(REP * h + 1) * DH]
                for r in range(1, REP):
                    qh = jnp.where(row == r, q[:, (REP * h + r) * DH:(REP * h + r + 1) * DH], qh)
                q_s[h] = qh

            def head(h, carry):
                k_copy(h).wait()
                s = jax.lax.dot_general(q_s[h].astype(bf16), k_v[h], _NT,
                                        preferred_element_type=f32)
                s = rnd(rnd(s) * sm_scale)
                m = jnp.max(s, axis=-1, keepdims=True)
                e = rnd(jnp.exp(rnd(s - m)))
                l = rnd(jnp.sum(e, axis=-1, keepdims=True))
                p = (e * (1.0 / l)).astype(bf16)
                v_copy(h).wait()
                o_s[h] = jax.lax.dot_general(p, v_v[h], _NN,
                                             preferred_element_type=f32)
                return carry

            jax.lax.fori_loop(0, HKV, head, 0)

            o_flat = jnp.concatenate(
                [o_s[h][r:r + 1, :] for h in range(HKV) for r in range(REP)], axis=1)
            o8 = jnp.broadcast_to(o_flat, (_SUB, HD)).astype(bf16)
            of_s[...] = o8.astype(f32)

            wg_cp.wait()
            g = jax.lax.dot_general(xn8, wg_v[...], _NN, preferred_element_type=f32)
            wu_cp.wait()
            u = jax.lax.dot_general(xn8, wu_v[...], _NN, preferred_element_type=f32)
            hh = (jax.nn.sigmoid(g) * u).astype(bf16)
            wd_cp.wait()
            y = jax.lax.dot_general(hh, wd_v[...], _NT, preferred_element_type=f32)
            gate = y * jax.nn.sigmoid(y)

            parts = []
            for i, (r0, r1) in enumerate(mxu_rows):
                wo_copy(i).wait()
                parts.append(jax.lax.dot_general(o8, wo_v[pl.ds(r0, r1 - r0), :], _NT,
                                                 preferred_element_type=f32))
            s_head = jnp.concatenate(parts, axis=1)
            res = x8[:, 0:R_TAIL] + s_head * gate[:, 0:R_TAIL]
            out_ref[0, :, 0:R_TAIL] = res[0:1].astype(out_ref.dtype)

            lane = jax.lax.broadcasted_iota(jnp.int32, (_SUB, N_TAIL), 1)
            sub = jax.lax.broadcasted_iota(jnp.int32, (_SUB, N_TAIL), 0)

            def place(acc, r, part):
                tot = jnp.sum(part, axis=-1, keepdims=True)
                return jnp.where(lane == sub + (r - R_TAIL), tot, acc)

            acc = jnp.zeros((_SUB, N_TAIL), f32)
            pending = []
            for i, (r0, r1) in enumerate(vpu_rows):
                wo_copy(len(mxu_rows) + i).wait()
                for r, part in pending:
                    acc = place(acc, r, part)
                pending = []
                for r in range(r0, r1, _SUB):
                    w = wo_v[pl.ds(r, _SUB), :].astype(f32)
                    pending.append((r, _tree_sum(
                        [w[:, c:c + _LANES] * of_s[:, c:c + _LANES] for c in range(0, HD, _LANES)])))
            for r, part in pending:
                acc = place(acc, r, part)
            s_tail = jnp.sum(acc, axis=0, keepdims=True)
            res_t = x[:, R_TAIL:] + s_tail * gate[0:1, R_TAIL:]
            out_ref[0, :, R_TAIL:D] = res_t.astype(out_ref.dtype)

        pl.run_scoped(main, pltpu.SemaphoreType.DMA((NSEM,)))

    scratch = [
        pltpu.VMEM((1, 1, D), bf16),
        pltpu.VMEM((D, HD), bf16),
        pltpu.VMEM((HKV, W, DH), bf16),
        pltpu.VMEM((HKV, W, DH), bf16),
        pltpu.VMEM((D, HD), bf16),
        pltpu.VMEM((D, F), bf16),
        pltpu.VMEM((D, F), bf16),
        pltpu.VMEM((D, F), bf16),
        pltpu.VMEM((HKV, _SUB, DH), f32),
        pltpu.VMEM((HKV, _SUB, DH), f32),
        pltpu.VMEM((_SUB, HD), f32),
    ]
    return kernel, scratch


@jax.jit
def pallas_recurrent_scan__sliding_block_cached__glu_gated_glu__decode_kernel(
    A_x: jax.Array,
    A_k_cache: jax.Array,
    A_v_cache: jax.Array,
    A_wq: jax.Array,
    A_wo: jax.Array,
    B_x: jax.Array,
    B_w_gate: jax.Array,
    B_w_up: jax.Array,
    B_w_down: jax.Array,
):
    _, _, D = A_x.shape
    _, HKV, SK, DH = A_k_cache.shape
    HQ = A_wq.shape[1] // DH
    F = B_w_gate.shape[1]
    kernel, scratch = _build(D, HQ, HKV, SK, DH, F)
    return pl.pallas_call(
        kernel,
        out_shape=jax.ShapeDtypeStruct(A_x.shape, A_x.dtype),
        in_specs=[pl.BlockSpec(memory_space=pl.ANY)] * 8,
        out_specs=pl.BlockSpec(memory_space=pltpu.VMEM),
        scratch_shapes=scratch,
        compiler_params=pltpu.CompilerParams(vmem_limit_bytes=100 * 1024 * 1024),
    )(A_x, A_wq, A_k_cache, A_v_cache, A_wo.T, B_w_gate, B_w_up, B_w_down.T)
```
